```python
import os as _os
_os.environ.setdefault("JAX_PLATFORMS", "cpu")
import jax
import jax.numpy as jnp

def _softmax(x, axis=-1):
    return jax.nn.softmax(x, axis=axis)
def _gelu(x):
    return jax.nn.gelu(x, approximate=True)
def _silu(x):
    return jax.nn.silu(x)
def _sigmoid(x):
    return jax.nn.sigmoid(x)
def _layernorm(x, axis=-1, eps=1e-5):
    m = jnp.mean(x, axis=axis, keepdims=True)
    v = jnp.var(x, axis=axis, keepdims=True)
    return (x - m) / jnp.sqrt(v + eps)
def _scatter_add(tgt, idx, src, axis=0):
    return tgt.at[idx].add(src)
def _segment_sum(src, seg, n):
    return jax.ops.segment_sum(src, seg, n)
class _Rng:
    def __init__(self, key):
        self._k = key
    def _next(self):
        self._k, sub = jax.random.split(self._k)
        return sub
    def normal(self, shape):
        return jax.random.normal(self._next(), shape, dtype=jnp.bfloat16)
    def randint(self, lo, hi, shape):
        return jax.random.randint(self._next(), shape, lo, hi, dtype=jnp.int32)
    def uniform(self, shape, lo=0.0, hi=1.0):
        return jax.random.uniform(self._next(), shape, jnp.bfloat16, lo, hi)
    def permutation(self, n):
        return jax.random.permutation(self._next(), n)


kernel_name = 'concat_heads__gqa_block_cached__mha_block_cached__near_ridge'

def setup_inputs():
    _rng = _Rng(jax.random.key(int.from_bytes(__import__("os").urandom(4), "little")))
    _w = (lambda a: (lambda t: t.astype(jnp.bfloat16) if jnp.issubdtype(t.dtype, jnp.floating) else t)(jnp.asarray(a)))
    def _A_setup():
        B, Sq, D = 16, 32, 512
        Hq, Hkv, Sk, Dh = 32, 8, 512, 128
        assert Hq % Hkv == 0, (Hq, Hkv)
        return {
            "x": _w((lambda *s: _rng.normal(s) * 0.8)(B, Sq, D)),
            "k_cache": _w((lambda *s: _rng.normal(s) * 0.8)(B, Hkv, Sk, Dh)),
            "v_cache": _w((lambda *s: _rng.normal(s) * 0.05)(B, Hkv, Sk, Dh)),
            "wq": _w((lambda *s: _rng.normal(s) * 0.8)(D, Hq * Dh) * (D ** -0.5)),
            "wo": _w((lambda *s: _rng.normal(s) * 0.05)(Hq * Dh, D) * ((Hq * Dh) ** -0.5)),
        }
    _A_in = _A_setup()

    def _B_setup():
        B, Sq, D = 16, 32, 512
        H, Sk, Dh = 32, 512, 128
        return {
            "x": _w((lambda *s: _rng.normal(s) * 0.8)(B, Sq, D)),
            "k_cache": _w((lambda *s: _rng.normal(s) * 0.8)(B, H, Sk, Dh)),
            "v_cache": _w((lambda *s: _rng.normal(s) * 0.05)(B, H, Sk, Dh)),
            "wq": _w((lambda *s: _rng.normal(s) * 0.8)(D, H * Dh) * (D ** -0.5)),
            "wo": _w((lambda *s: _rng.normal(s) * 0.05)(H * Dh, D) * ((H * Dh) ** -0.5)),
        }
    _B_in = _B_setup()

    return {
        "A_x": _A_in["x"],
        "A_k_cache": _A_in["k_cache"],
        "A_v_cache": _A_in["v_cache"],
        "A_wq": _A_in["wq"],
        "A_wo": _A_in["wo"],
        "B_x": _B_in["x"],
        "B_k_cache": _B_in["k_cache"],
        "B_v_cache": _B_in["v_cache"],
        "B_wq": _B_in["wq"],
        "B_wo": _B_in["wo"],
    }

def reference(A_x, A_k_cache, A_v_cache, A_wq, A_wo, B_x, B_k_cache, B_v_cache, B_wq, B_wo):
    def _A_ref(x, k_cache, v_cache, wq, wo):
        B, Sq, D = x.shape
        Hq, Dh = 32, 128
        Hkv = k_cache.shape[1]
        rep = Hq // Hkv
        q = (lambda x, *d: x.transpose(*d))((x @ wq).reshape(B, Sq, Hq, Dh), 0, 2, 1, 3)
        k = jnp.repeat(k_cache, rep, axis=1)
        v = jnp.repeat(v_cache, rep, axis=1)
        scores = jnp.einsum("bhqd,bhkd->bhqk", q, k) * (Dh ** -0.5)
        p = _softmax(scores, axis=-1)
        o = jnp.einsum("bhqk,bhkd->bhqd", p, v)
        return (lambda x, *d: x.transpose(*d))(o, 0, 2, 1, 3).reshape(B, Sq, Hq * Dh) @ wo

    def _B_ref(x, k_cache, v_cache, wq, wo):
        B, Sq, D = x.shape
        H, Dh = 32, 128
        q = (lambda x, *d: x.transpose(*d))((x @ wq).reshape(B, Sq, H, Dh), 0, 2, 1, 3)
        scores = jnp.einsum("bhqd,bhkd->bhqk", q, k_cache) * (Dh ** -0.5)
        p = _softmax(scores, axis=-1)
        o = jnp.einsum("bhqk,bhkd->bhqd", p, v_cache)
        return (lambda x, *d: x.transpose(*d))(o, 0, 2, 1, 3).reshape(B, Sq, H * Dh) @ wo

    a = _A_ref(A_x, A_k_cache, A_v_cache, A_wq, A_wo)
    b = _B_ref(B_x, B_k_cache, B_v_cache, B_wq, B_wo)
    return jnp.concatenate([a, b], axis=-1)
```

```python
import numpy as np

import jax
import jax.numpy as jnp
from jax import lax
import jax.experimental.pallas as pl
import jax.experimental.pallas.tpu as pltpu

B, SQ, D = 16, 32, 512
HQ, HKV, SK, DH = 32, 8, 512, 128
REP = HQ // HKV
M = B * SQ
G = HKV
GW = REP * DH
NB = 4
NC = B // NB
R = NB * SQ
QSCALE = float(DH ** -0.5 * np.log2(np.e))


def _kernel(xa_h, ka_h, va_h, wqa_h, woa_h, xb_h, kb_h, vb_h, wqb_h, wob_h,
            out_h,
            x_buf, wq_buf, wo_buf, ka_buf, va_buf, kb_buf, vb_buf, acc, obuf,
            sem_a, sem_k, sem_v, sem_o):

  def group_cols(g):
    return pl.ds(pl.multiple_of(g * GW, GW), GW)

  def x_copies():
    return (pltpu.make_async_copy(xa_h, x_buf.at[0], sem_a),
            pltpu.make_async_copy(xb_h, x_buf.at[1], sem_a))

  def a_copies(g):
    return (pltpu.make_async_copy(wqa_h.at[:, group_cols(g)], wq_buf.at[0, g], sem_a),
            pltpu.make_async_copy(ka_h.at[:, g], ka_buf, sem_a),
            pltpu.make_async_copy(va_h.at[:, g], va_buf, sem_a),
            pltpu.make_async_copy(woa_h.at[group_cols(g), :], wo_buf.at[0, g], sem_a))

  def k_copy(g, c):
    return pltpu.make_async_copy(
        kb_h.at[pl.ds(c * NB, NB), pl.ds(g * REP, REP)], kb_buf.at[c], sem_k.at[c])

  def v_copy(g, c):
    return pltpu.make_async_copy(
        vb_h.at[pl.ds(c * NB, NB), pl.ds(g * REP, REP)], vb_buf.at[c], sem_v.at[c])

  def wqb_copy(g):
    return pltpu.make_async_copy(wqb_h.at[:, group_cols(g)], wq_buf.at[1, g], sem_k.at[0])

  def wob_copy(g):
    return pltpu.make_async_copy(wob_h.at[group_cols(g), :], wo_buf.at[1, g], sem_v.at[0])

  def out_copies():
    head, tail = pl.ds(0, M - R), pl.ds(M - R, R)
    cols_a, cols_b = pl.ds(0, D), pl.ds(D, D)
    return (pltpu.make_async_copy(obuf.at[:, cols_a], out_h.at[:, cols_a], sem_o),
            pltpu.make_async_copy(obuf.at[head, cols_b], out_h.at[head, cols_b], sem_o),
            pltpu.make_async_copy(obuf.at[tail, cols_b], out_h.at[tail, cols_b], sem_o))

  def qk(q, k):
    return lax.dot_general(q, k, (((1,), (1,)), ((), ())),
                           preferred_element_type=jnp.float32)

  def softmax(s):
    p = jnp.exp2(s - jnp.max(s, axis=-1, keepdims=True))
    return p.astype(jnp.bfloat16), 1.0 / jnp.sum(p, axis=-1, keepdims=True)

  def pv(p, r, v):
    return (jnp.dot(p, v, preferred_element_type=jnp.float32) * r).astype(jnp.bfloat16)

  def q_proj(br, g, rows):
    q = jnp.dot(x_buf[br, rows, :], wq_buf[br, g], preferred_element_type=jnp.float32)
    return (q * QSCALE).astype(jnp.bfloat16)

  def o_proj(br, g, rows, o):
    r = acc[br, rows, :] + jnp.dot(o, wo_buf[br, g], preferred_element_type=jnp.float32)
    acc[br, rows, :] = r
    obuf[rows, br * D:(br + 1) * D] = r.astype(jnp.bfloat16)

  for cp in x_copies() + a_copies(0) + (wqb_copy(0), wob_copy(0)):
    cp.start()
  for c in range(NC):
    k_copy(0, c).start()
    v_copy(0, c).start()

  acc[...] = jnp.zeros_like(acc)
  for cp in x_copies():
    cp.wait()

  def group(g, carry):
    more = g + 1 < G

    for cp in a_copies(g):
      cp.wait()

    def a_chunk(c, carry):
      rows = pl.ds(pl.multiple_of(c * R, R), R)
      q = q_proj(0, g, rows)
      ps = []
      for i in range(NB):
        qi = jnp.concatenate(
            [q[i * SQ:(i + 1) * SQ, h * DH:(h + 1) * DH] for h in range(REP)], axis=0)
        ps.append(softmax(qk(qi, ka_buf[c * NB + i])))
      outs = []
      for i in range(NB):
        o = pv(*ps[i], va_buf[c * NB + i])
        outs.append(jnp.concatenate([o[h * SQ:(h + 1) * SQ] for h in range(REP)], axis=1))
      o_proj(0, g, rows, jnp.concatenate(outs, axis=0))
      return carry

    lax.fori_loop(0, NC, a_chunk, 0)

    @pl.when(more)
    def _():
      for cp in a_copies(g + 1):
        cp.start()

    def b_chunk(c, carry):
      @pl.when(c == 0)
      def _():
        wqb_copy(g).wait()

      k_copy(g, c).wait()
      rows = pl.ds(pl.multiple_of(c * R, R), R)
      q = q_proj(1, g, rows)
      ps = []
      for i in range(NB):
        for h in range(REP):
          ps.append(softmax(qk(q[i * SQ:(i + 1) * SQ, h * DH:(h + 1) * DH], kb_buf[c, i, h])))

      @pl.when(c == 0)
      def _():
        wob_copy(g).wait()

      v_copy(g, c).wait()

      @pl.when(jnp.logical_and(g == G - 1, c == NC - 1))
      def _():
        for cp in out_copies()[:2]:
          cp.start()

      outs = []
      for i in range(NB):
        outs.append(jnp.concatenate(
            [pv(*ps[i * REP + h], vb_buf[c, i, h]) for h in range(REP)], axis=1))
      o_proj(1, g, rows, jnp.concatenate(outs, axis=0))

      @pl.when(more)
      def _():
        @pl.when(c == 0)
        def _():
          wqb_copy(g + 1).start()
          wob_copy(g + 1).start()

        k_copy(g + 1, c).start()
        v_copy(g + 1, c).start()

      return carry

    lax.fori_loop(0, NC, b_chunk, 0)
    return carry

  lax.fori_loop(0, G, group, 0)

  out_copies()[2].start()
  for cp in out_copies():
    cp.wait()


@jax.jit
def pallas_concat_heads__gqa_block_cached__mha_block_cached__near_ridge_kernel(
    A_x: jax.Array,
    A_k_cache: jax.Array,
    A_v_cache: jax.Array,
    A_wq: jax.Array,
    A_wo: jax.Array,
    B_x: jax.Array,
    B_k_cache: jax.Array,
    B_v_cache: jax.Array,
    B_wq: jax.Array,
    B_wo: jax.Array,
):
  hbm = pl.BlockSpec(memory_space=pltpu.HBM)
  out = pl.pallas_call(
      _kernel,
      out_shape=jax.ShapeDtypeStruct((M, 2 * D), jnp.bfloat16),
      in_specs=[hbm] * 10,
      out_specs=hbm,
      scratch_shapes=[
          pltpu.VMEM((2, M, D), jnp.bfloat16),
          pltpu.VMEM((2, G, D, GW), jnp.bfloat16),
          pltpu.VMEM((2, G, GW, D), jnp.bfloat16),
          pltpu.VMEM((B, SK, DH), jnp.bfloat16),
          pltpu.VMEM((B, SK, DH), jnp.bfloat16),
          pltpu.VMEM((NC, NB, REP, SK, DH), jnp.bfloat16),
          pltpu.VMEM((NC, NB, REP, SK, DH), jnp.bfloat16),
          pltpu.VMEM((2, M, D), jnp.float32),
          pltpu.VMEM((M, 2 * D), jnp.bfloat16),
          pltpu.SemaphoreType.DMA(()),
          pltpu.SemaphoreType.DMA((NC,)),
          pltpu.SemaphoreType.DMA((NC,)),
          pltpu.SemaphoreType.DMA(()),
      ],
      compiler_params=pltpu.CompilerParams(vmem_limit_bytes=100 * 1024 * 1024),
  )(A_x.reshape(M, D), A_k_cache, A_v_cache, A_wq, A_wo,
    B_x.reshape(M, D), B_k_cache, B_v_cache, B_wq, B_wo)
  return out.reshape(B, SQ, 2 * D)
```

```python
import functools

import numpy as np

import jax
import jax.numpy as jnp
from jax import lax
import jax.experimental.pallas as pl
import jax.experimental.pallas.tpu as pltpu

B, SQ, D = 16, 32, 512
HQ, HKV, SK, DH = 32, 8, 512, 128
REP = HQ // HKV
G = HKV
GW = REP * DH
M = B * SQ

P = 8
NA = B // P
NB = B * REP // P
NJ = NA + NB
A_BATCH = 4
B_BATCH = P // REP
NSL = 4
SL = SK // NSL
AHEAD = 3
STAGED_A = (3, 2)
STAGED_B = 2
NSTAGE = 4

QSCALE = float(DH ** -0.5 * np.log2(np.e))


def _start_all(copies):
  for cp in copies:
    cp.start()


def _wait_all(copies):
  for cp in copies:
    cp.wait()


def _qk(q, k):
  return lax.dot_general(q, k, (((1,), (1,)), ((), ())),
                         preferred_element_type=jnp.float32)


def _softmax(s):
  p = jnp.exp2(s - jnp.max(s, axis=-1, keepdims=True))
  return p.astype(jnp.bfloat16), 1.0 / jnp.sum(p, axis=-1, keepdims=True)


def _pv(p, r, v):
  return (jnp.dot(p, v, preferred_element_type=jnp.float32) * r).astype(jnp.bfloat16)


def _kernel(xa_h, ka_h, va_h, wqa_h, woa_h, xb_h, kb_h, vb_h, wqb_h, wob_h,
            out_h,
            x_buf, wq_buf, woa_buf, wob_buf, k_buf, v_buf, acc, obuf, sbuf,
            sem_o):

  def out_copy(last):
    n = B_BATCH * SQ
    rows = pl.ds(M - n, n) if last else pl.ds(0, M - n)
    return pltpu.make_async_copy(obuf.at[rows], out_h.at[rows], sem_o)

  def body(sem_x, sem_k, sem_v, sem_l, sem_in, sem_fw):

    def group_cols(g):
      return pl.ds(pl.multiple_of(g * GW, GW), GW)

    def head_cols(g, h):
      return pl.ds(pl.multiple_of((g + G * h) * DH, DH), DH)

    def slot(br, t):
      return t if br == 0 else NA + t

    def staged(br, t):
      return STAGED_A[t] if br == 0 else STAGED_B

    def x_copy(br):
      return pltpu.make_async_copy((xa_h, xb_h)[br], x_buf.at[br], sem_x.at[br])

    def wq_copies(g, br):
      if br == 0:
        return [pltpu.make_async_copy(
            wqa_h.at[:, group_cols(g)], wq_buf.at[0, :, group_cols(g)], sem_k.at[0])]
      return [pltpu.make_async_copy(
          wqb_h.at[:, head_cols(g, h)], wq_buf.at[1, :, head_cols(g, h)], sem_k.at[NA])
              for h in range(REP)]

    def wo_copy(g, br):
      if br == 0:
        return pltpu.make_async_copy(
            woa_h.at[group_cols(g), :], woa_buf.at[group_cols(g), :], sem_v.at[0])
      return pltpu.make_async_copy(wob_h.at[:, g], wob_buf.at[:, g], sem_v.at[NA])

    def k_copies(g, br, t):
      j = slot(br, t)
      return [pltpu.make_async_copy(
          (ka_h, kb_h)[br].at[pl.ds(t * P, P), g, pl.ds(s * SL, SL)],
          k_buf.at[j, :, pl.ds(s * SL, SL)], sem_k.at[j]) for s in range(NSL)]

    def v_copy(g, br, t, s):
      j = slot(br, t)
      n = P - 1 if s >= NSL - staged(br, t) else P
      sem = sem_l if s == NSL - 1 else sem_v
      return pltpu.make_async_copy(
          (va_h, vb_h)[br].at[pl.ds(t * P, n), g, pl.ds(s * SL, SL)],
          v_buf.at[j, pl.ds(0, n), pl.ds(s * SL, SL)], sem.at[j])

    def stage_in(g, br, t):
      n = g * NJ + slot(br, t)
      r = staged(br, t) * SL
      return pltpu.make_async_copy(
          (va_h, vb_h)[br].at[t * P + P - 1, g, pl.ds(SK - r, r)],
          sbuf.at[n % NSTAGE, pl.ds(0, r)], sem_in.at[n % 2])

    def stage_out(g, br, t):
      j = slot(br, t)
      n = g * NJ + j
      r = staged(br, t) * SL
      return pltpu.make_async_copy(
          sbuf.at[n % NSTAGE, pl.ds(0, r)],
          v_buf.at[j, P - 1, pl.ds(SK - r, r)], sem_fw.at[n % 2])

    def on_first(t, fn):
      if isinstance(t, int):
        if t == 0:
          fn()
      else:
        pl.when(t == 0)(fn)

    def start_k(g, br, t):
      on_first(t, lambda: _start_all(wq_copies(g, br)))
      _start_all(k_copies(g, br, t))

    def start_v(g, br, t):
      on_first(t, lambda: wo_copy(g, br).start())
      for s in range(NSL - 1):
        v_copy(g, br, t, s).start()

    def start_v_last(g, br, t):
      v_copy(g, br, t, NSL - 1).start()

    def start_stage(g, br, t):
      stage_in(g, br, t).start()

    def forward_stage(g, br, t):
      stage_in(g, br, t).wait()
      stage_out(g, br, t).start()

    def later(g, br, t, d, fn):
      if br == 0:
        j = t + d
        if j < NA:
          fn(g, 0, j)
        else:
          fn(g, 1, j - NA)
        return
      pl.when(t + d < NB)(lambda: fn(g, 1, t + d))

      @pl.when(g + 1 < G)
      def _():
        for a in range(min(NA, d)):
          pl.when(t + d == NB + a)(functools.partial(fn, g + 1, 0, a))
        if d > NA:
          pl.when(t + d >= NJ)(lambda: fn(g + 1, 1, t + d - NJ))

    def wait_k(g, br, t):
      on_first(t, lambda: _wait_all(wq_copies(g, br)))
      _wait_all(k_copies(g, br, t))
      later(g, br, t, AHEAD, start_k)

    def wait_v(g, br, t):
      on_first(t, lambda: wo_copy(g, br).wait())
      for s in range(NSL - 1):
        v_copy(g, br, t, s).wait()
      if br == 1:
        pl.when(jnp.logical_and(g == G - 1, t == NB - 1))(lambda: out_copy(False).start())
      later(g, br, t, AHEAD, start_v)
      stage_out(g, br, t).wait()
      later(g, br, t, 2, forward_stage)
      later(g, br, t, NSTAGE, start_stage)
      v_copy(g, br, t, NSL - 1).wait()
      later(g, br, t, AHEAD, start_v_last)

    def q_proj(br, g, rows):
      if br == 0:
        w = wq_buf[0, :, group_cols(g)]
      else:
        w = jnp.concatenate([wq_buf[1, :, head_cols(g, h)] for h in range(REP)], axis=1)
      q = jnp.dot(x_buf[br, rows, :], w, preferred_element_type=jnp.float32)
      return (q * QSCALE).astype(jnp.bfloat16)

    def o_proj(br, g, rows, o):
      if br == 0:
        w = woa_buf[group_cols(g), :]
      else:
        w = jnp.concatenate([wob_buf[h, g] for h in range(REP)], axis=0)
      r = acc[br, rows, :] + jnp.dot(o, w, preferred_element_type=jnp.float32)
      acc[br, rows, :] = r
      obuf[rows, br * D:(br + 1) * D] = r.astype(jnp.bfloat16)

    def a_compute(g, t, c, carry):
      n = A_BATCH * SQ
      rows = pl.ds(pl.multiple_of(t * P * SQ + c * n, n), n)
      q = q_proj(0, g, rows)
      ps = []
      for i in range(A_BATCH):
        qi = jnp.concatenate(
            [q[i * SQ:(i + 1) * SQ, h * DH:(h + 1) * DH] for h in range(REP)], axis=0)
        ps.append(_softmax(_qk(qi, k_buf[t, c * A_BATCH + i])))
      outs = []
      for i in range(A_BATCH):
        o = _pv(*ps[i], v_buf[t, c * A_BATCH + i])
        outs.append(jnp.concatenate([o[h * SQ:(h + 1) * SQ] for h in range(REP)], axis=1))
      o_proj(0, g, rows, jnp.concatenate(outs, axis=0))
      return carry

    def b_step(g, t, carry):
      j = NA + t
      n = B_BATCH * SQ
      rows = pl.ds(pl.multiple_of(t * n, n), n)
      wait_k(g, 1, t)
      q = q_proj(1, g, rows)
      ps = [_softmax(_qk(q[i * SQ:(i + 1) * SQ, h * DH:(h + 1) * DH], k_buf[j, i * REP + h]))
            for i in range(B_BATCH) for h in range(REP)]
      wait_v(g, 1, t)
      outs = [jnp.concatenate(
          [_pv(*ps[i * REP + h], v_buf[j, i * REP + h]) for h in range(REP)], axis=1)
              for i in range(B_BATCH)]
      o_proj(1, g, rows, jnp.concatenate(outs, axis=0))
      return carry

    def group(g, carry):
      for t in range(NA):
        wait_k(g, 0, t)
        wait_v(g, 0, t)
        lax.fori_loop(0, P // A_BATCH, functools.partial(a_compute, g, t), 0)
      pl.when(g == 0)(lambda: x_copy(1).wait())
      lax.fori_loop(0, NB, functools.partial(b_step, g), 0)
      return carry

    first = [(0, 0, j) if j < NA else (0, 1, j - NA) for j in range(NJ)]
    start_stage(*first[0])
    start_stage(*first[1])
    x_copy(0).start()
    for j in range(AHEAD):
      start_k(*first[j])
      start_v(*first[j])
      start_v_last(*first[j])
    x_copy(1).start()
    acc[...] = jnp.zeros_like(acc)
    for j in range(2):
      forward_stage(*first[j])
      start_stage(*first[j + 2])
    x_copy(0).wait()

    lax.fori_loop(0, G, group, 0)
    out_copy(True).start()

  dma = pltpu.SemaphoreType.DMA
  pl.run_scoped(body, dma((2,)), dma((NJ,)), dma((NJ,)), dma((NJ,)), dma((2,)), dma((2,)))
  out_copy(False).wait()
  out_copy(True).wait()


@jax.jit
def pallas_concat_heads__gqa_block_cached__mha_block_cached__near_ridge_kernel(
    A_x: jax.Array,
    A_k_cache: jax.Array,
    A_v_cache: jax.Array,
    A_wq: jax.Array,
    A_wo: jax.Array,
    B_x: jax.Array,
    B_k_cache: jax.Array,
    B_v_cache: jax.Array,
    B_wq: jax.Array,
    B_wo: jax.Array,
):
  hbm = pl.BlockSpec(memory_space=pltpu.HBM)
  out = pl.pallas_call(
      _kernel,
      out_shape=jax.ShapeDtypeStruct((M, 2 * D), jnp.bfloat16),
      in_specs=[hbm] * 10,
      out_specs=hbm,
      scratch_shapes=[
          pltpu.VMEM((2, M, D), jnp.bfloat16),
          pltpu.VMEM((2, D, HQ * DH), jnp.bfloat16),
          pltpu.VMEM((HQ * DH, D), jnp.bfloat16),
          pltpu.VMEM((REP, G, DH, D), jnp.bfloat16),
          pltpu.VMEM((NJ, P, SK, DH), jnp.bfloat16),
          pltpu.VMEM((NJ, P, SK, DH), jnp.bfloat16),
          pltpu.VMEM((2, M, D), jnp.float32),
          pltpu.VMEM((M, 2 * D), jnp.bfloat16),
          pltpu.SMEM((NSTAGE, max(STAGED_A + (STAGED_B,)) * SL, DH), jnp.bfloat16),
          pltpu.SemaphoreType.DMA(()),
      ],
      compiler_params=pltpu.CompilerParams(vmem_limit_bytes=100 * 1024 * 1024),
  )(A_x.reshape(M, D), A_k_cache, A_v_cache, A_wq, A_wo,
    B_x.reshape(M, D),
    B_k_cache.reshape(B * REP, G, SK, DH), B_v_cache.reshape(B * REP, G, SK, DH),
    B_wq, B_wo.reshape(REP, G, DH, D))
  return out.reshape(B, SQ, 2 * D)
```

```python
import functools

import numpy as np

import jax
import jax.numpy as jnp
from jax import lax
import jax.experimental.pallas as pl
import jax.experimental.pallas.tpu as pltpu

B, SQ, D = 16, 32, 512
HQ, HKV, SK, DH = 32, 8, 512, 128
REP = HQ // HKV
G = HKV
GW = REP * DH
M = B * SQ

P = 8
NA = B // P
NB = B * REP // P
NJ = NA + NB
A_BATCH = 4
B_BATCH = P // REP
NSL = 4
SL = SK // NSL
AHEAD = 3
STAGED = (288, 272)
DEPTH = 3

QSCALE = float(DH ** -0.5 * np.log2(np.e))


def _start_all(copies):
  for cp in copies:
    cp.start()


def _wait_all(copies):
  for cp in copies:
    cp.wait()


def _qk(q, k):
  return lax.dot_general(q, k, (((1,), (1,)), ((), ())),
                         preferred_element_type=jnp.float32)


def _softmax(s):
  p = jnp.exp2(s - jnp.max(s, axis=-1, keepdims=True))
  return p.astype(jnp.bfloat16), 1.0 / jnp.sum(p, axis=-1, keepdims=True)


def _pv(p, r, v):
  return (jnp.dot(p, v, preferred_element_type=jnp.float32) * r).astype(jnp.bfloat16)


def _kernel(xa_h, ka_h, va_h, wqa_h, woa_h, xb_h, kb_h, vb_h, wqb_h, wob_h,
            out_h,
            x_buf, wq_buf, woa_buf, wob_buf, k_buf, v_buf, acc, obuf, sbuf,
            sem_o):

  def out_copy(last):
    n = B_BATCH * SQ
    rows = pl.ds(M - n, n) if last else pl.ds(0, M - n)
    return pltpu.make_async_copy(obuf.at[rows], out_h.at[rows], sem_o)

  def body(sem_x, sem_k, sem_v, sem_l, sem_in, sem_fw):

    def group_cols(g):
      return pl.ds(pl.multiple_of(g * GW, GW), GW)

    def head_cols(g, h):
      return pl.ds(pl.multiple_of((g + G * h) * DH, DH), DH)

    def slot(br, t):
      return t if br == 0 else NA + t

    def x_copy(br):
      return pltpu.make_async_copy((xa_h, xb_h)[br], x_buf.at[br], sem_x.at[br])

    def wq_copies(g, br):
      if br == 0:
        return [pltpu.make_async_copy(
            wqa_h.at[:, group_cols(g)], wq_buf.at[0, :, group_cols(g)], sem_k.at[0])]
      return [pltpu.make_async_copy(
          wqb_h.at[:, head_cols(g, h)], wq_buf.at[1, :, head_cols(g, h)], sem_k.at[NA])
              for h in range(REP)]

    def wo_copy(g, br):
      if br == 0:
        return pltpu.make_async_copy(
            woa_h.at[group_cols(g), :], woa_buf.at[group_cols(g), :], sem_v.at[0])
      return pltpu.make_async_copy(wob_h.at[:, g], wob_buf.at[:, g], sem_v.at[NA])

    def k_copies(g, br, t):
      j = slot(br, t)
      return [pltpu.make_async_copy(
          (ka_h, kb_h)[br].at[pl.ds(t * P, P), g, pl.ds(s * SL, SL)],
          k_buf.at[j, :, pl.ds(s * SL, SL)], sem_k.at[j]) for s in range(NSL)]

    def v_copies(g, br, t):
      j = slot(br, t)
      kept = SK - STAGED[br]

      def copy(block, blocks, row, rows, sem):
        return pltpu.make_async_copy(
            (va_h, vb_h)[br].at[pl.ds(t * P + block, blocks), g, pl.ds(row, rows)],
            v_buf.at[j, pl.ds(block, blocks), pl.ds(row, rows)], sem.at[j])

      copies = []
      for s in range(NSL):
        row = s * SL
        sem = sem_l if s == NSL - 1 else sem_v
        if row + SL <= kept:
          copies.append(copy(0, P, row, SL, sem))
        else:
          if row < kept:
            copies.append(copy(P - 1, 1, row, kept - row, sem_v))
          copies.append(copy(0, P - 1, row, SL, sem))
      return copies

    def stage_in(g, br, t):
      n = g * NJ + slot(br, t)
      r = STAGED[br]
      return pltpu.make_async_copy(
          (va_h, vb_h)[br].at[t * P + P - 1, g, pl.ds(SK - r, r)],
          sbuf.at[n % (2 * DEPTH), pl.ds(0, r)], sem_in.at[n % DEPTH])

    def stage_out(g, br, t):
      j = slot(br, t)
      n = g * NJ + j
      r = STAGED[br]
      return pltpu.make_async_copy(
          sbuf.at[n % (2 * DEPTH), pl.ds(0, r)],
          v_buf.at[j, P - 1, pl.ds(SK - r, r)], sem_fw.at[n % DEPTH])

    def on_first(t, fn):
      if isinstance(t, int):
        if t == 0:
          fn()
      else:
        pl.when(t == 0)(fn)

    def start_k(g, br, t):
      on_first(t, lambda: _start_all(wq_copies(g, br)))
      _start_all(k_copies(g, br, t))

    def start_v(g, br, t):
      on_first(t, lambda: wo_copy(g, br).start())
      _start_all(v_copies(g, br, t)[:-1])

    def start_v_last(g, br, t):
      v_copies(g, br, t)[-1].start()

    def start_stage(g, br, t):
      stage_in(g, br, t).start()

    def forward_stage(g, br, t):
      stage_in(g, br, t).wait()
      stage_out(g, br, t).start()

    def later(g, br, t, d, fn):
      if br == 0:
        j = t + d
        if j < NA:
          fn(g, 0, j)
        else:
          fn(g, 1, j - NA)
        return
      pl.when(t + d < NB)(lambda: fn(g, 1, t + d))

      @pl.when(g + 1 < G)
      def _():
        for a in range(min(NA, d)):
          pl.when(t + d == NB + a)(functools.partial(fn, g + 1, 0, a))
        if d > NA:
          pl.when(t + d >= NJ)(lambda: fn(g + 1, 1, t + d - NJ))

    def wait_k(g, br, t):
      on_first(t, lambda: _wait_all(wq_copies(g, br)))
      _wait_all(k_copies(g, br, t))
      later(g, br, t, AHEAD, start_k)

    def wait_v(g, br, t):
      on_first(t, lambda: wo_copy(g, br).wait())
      copies = v_copies(g, br, t)
      _wait_all(copies[:-1])
      if br == 1:
        pl.when(jnp.logical_and(g == G - 1, t == NB - 1))(lambda: out_copy(False).start())
      later(g, br, t, AHEAD, start_v)
      stage_out(g, br, t).wait()
      later(g, br, t, DEPTH, forward_stage)
      later(g, br, t, 2 * DEPTH, start_stage)
      copies[-1].wait()
      later(g, br, t, AHEAD, start_v_last)

    def q_proj(br, g, rows):
      if br == 0:
        w = wq_buf[0, :, group_cols(g)]
      else:
        w = jnp.concatenate([wq_buf[1, :, head_cols(g, h)] for h in range(REP)], axis=1)
      q = jnp.dot(x_buf[br, rows, :], w, preferred_element_type=jnp.float32)
      return (q * QSCALE).astype(jnp.bfloat16)

    def o_proj(br, g, rows, o):
      if br == 0:
        w = woa_buf[group_cols(g), :]
      else:
        w = jnp.concatenate([wob_buf[h, g] for h in range(REP)], axis=0)
      r = acc[br, rows, :] + jnp.dot(o, w, preferred_element_type=jnp.float32)
      acc[br, rows, :] = r
      obuf[rows, br * D:(br + 1) * D] = r.astype(jnp.bfloat16)

    def a_compute(g, t, c, carry):
      n = A_BATCH * SQ
      rows = pl.ds(pl.multiple_of(t * P * SQ + c * n, n), n)
      q = q_proj(0, g, rows)
      ps = []
      for i in range(A_BATCH):
        qi = jnp.concatenate(
            [q[i * SQ:(i + 1) * SQ, h * DH:(h + 1) * DH] for h in range(REP)], axis=0)
        ps.append(_softmax(_qk(qi, k_buf[t, c * A_BATCH + i])))
      outs = []
      for i in range(A_BATCH):
        o = _pv(*ps[i], v_buf[t, c * A_BATCH + i])
        outs.append(jnp.concatenate([o[h * SQ:(h + 1) * SQ] for h in range(REP)], axis=1))
      o_proj(0, g, rows, jnp.concatenate(outs, axis=0))
      return carry

    def b_step(g, t, carry):
      j = NA + t
      n = B_BATCH * SQ
      rows = pl.ds(pl.multiple_of(t * n, n), n)
      wait_k(g, 1, t)
      q = q_proj(1, g, rows)
      ps = [_softmax(_qk(q[i * SQ:(i + 1) * SQ, h * DH:(h + 1) * DH], k_buf[j, i * REP + h]))
            for i in range(B_BATCH) for h in range(REP)]
      wait_v(g, 1, t)
      outs = [jnp.concatenate(
          [_pv(*ps[i * REP + h], v_buf[j, i * REP + h]) for h in range(REP)], axis=1)
              for i in range(B_BATCH)]
      o_proj(1, g, rows, jnp.concatenate(outs, axis=0))
      return carry

    def group(g, carry):
      for t in range(NA):
        wait_k(g, 0, t)
        wait_v(g, 0, t)
        lax.fori_loop(0, P // A_BATCH, functools.partial(a_compute, g, t), 0)
      pl.when(g == 0)(lambda: x_copy(1).wait())
      lax.fori_loop(0, NB, functools.partial(b_step, g), 0)
      return carry

    first = [(0, 0, j) if j < NA else (0, 1, j - NA) for j in range(NJ)]
    for j in range(DEPTH):
      start_stage(*first[j])
    x_copy(0).start()
    for j in range(AHEAD):
      start_k(*first[j])
      start_v(*first[j])
      start_v_last(*first[j])
    x_copy(1).start()
    acc[...] = jnp.zeros_like(acc)
    for j in range(DEPTH):
      forward_stage(*first[j])
      start_stage(*first[j + DEPTH])
    x_copy(0).wait()

    lax.fori_loop(0, G, group, 0)
    out_copy(True).start()

  dma = pltpu.SemaphoreType.DMA
  pl.run_scoped(body, dma((2,)), dma((NJ,)), dma((NJ,)), dma((NJ,)), dma((DEPTH,)), dma((DEPTH,)))
  out_copy(False).wait()
  out_copy(True).wait()


@jax.jit
def pallas_concat_heads__gqa_block_cached__mha_block_cached__near_ridge_kernel(
    A_x: jax.Array,
    A_k_cache: jax.Array,
    A_v_cache: jax.Array,
    A_wq: jax.Array,
    A_wo: jax.Array,
    B_x: jax.Array,
    B_k_cache: jax.Array,
    B_v_cache: jax.Array,
    B_wq: jax.Array,
    B_wo: jax.Array,
):
  hbm = pl.BlockSpec(memory_space=pltpu.HBM)
  out = pl.pallas_call(
      _kernel,
      out_shape=jax.ShapeDtypeStruct((M, 2 * D), jnp.bfloat16),
      in_specs=[hbm] * 10,
      out_specs=hbm,
      scratch_shapes=[
          pltpu.VMEM((2, M, D), jnp.bfloat16),
          pltpu.VMEM((2, D, HQ * DH), jnp.bfloat16),
          pltpu.VMEM((HQ * DH, D), jnp.bfloat16),
          pltpu.VMEM((REP, G, DH, D), jnp.bfloat16),
          pltpu.VMEM((NJ, P, SK, DH), jnp.bfloat16),
          pltpu.VMEM((NJ, P, SK, DH), jnp.bfloat16),
          pltpu.VMEM((2, M, D), jnp.float32),
          pltpu.VMEM((M, 2 * D), jnp.bfloat16),
          pltpu.SMEM((2 * DEPTH, max(STAGED), DH), jnp.bfloat16),
          pltpu.SemaphoreType.DMA(()),
      ],
      compiler_params=pltpu.CompilerParams(
          vmem_limit_bytes=100 * 1024 * 1024, disable_bounds_checks=True),
  )(A_x.reshape(M, D), A_k_cache, A_v_cache, A_wq, A_wo,
    B_x.reshape(M, D),
    B_k_cache.reshape(B * REP, G, SK, DH), B_v_cache.reshape(B * REP, G, SK, DH),
    B_wq, B_wo.reshape(REP, G, DH, D))
  return out.reshape(B, SQ, 2 * D)
```

```python
import functools

import numpy as np

import jax
import jax.numpy as jnp
from jax import lax
import jax.experimental.pallas as pl
import jax.experimental.pallas.tpu as pltpu

B, SQ, D = 16, 32, 512
HQ, HKV, SK, DH = 32, 8, 512, 128
REP = HQ // HKV
G = HKV
GW = REP * DH
M = B * SQ

P = 8
NA = B // P
NB = B * REP // P
NJ = NA + NB
A_BATCH = 4
B_BATCH = P // REP
NSL = 4
SL = SK // NSL
AHEAD = 3
STAGED = (288, 272)
DEPTH = 3

QSCALE = float(DH ** -0.5 * np.log2(np.e))


def _start_all(copies):
  for cp in copies:
    cp.start()


def _wait_all(copies):
  for cp in copies:
    cp.wait()


def _qk(q, k):
  return lax.dot_general(q, k, (((1,), (1,)), ((), ())),
                         preferred_element_type=jnp.float32)


def _softmax(s):
  p = jnp.exp2(s - jnp.max(s, axis=-1, keepdims=True))
  return p.astype(jnp.bfloat16), 1.0 / jnp.sum(p, axis=-1, keepdims=True)


def _pv(p, r, v):
  return (jnp.dot(p, v, preferred_element_type=jnp.float32) * r).astype(jnp.bfloat16)


def _kernel(xa_h, ka_h, va_h, wqa_h, woa_h, xb_h, kb_h, vb_h, wqb_h, wob_h,
            out_h,
            x_buf, wq_buf, woa_buf, wob_buf, k_buf, v_buf, acc, obuf, sbuf,
            sem_o):

  def out_copy(last):
    n = B_BATCH * SQ
    rows = pl.ds(M - n, n) if last else pl.ds(0, M - n)
    return pltpu.make_async_copy(obuf.at[rows], out_h.at[rows], sem_o)

  def body(sem_x, sem_k, sem_v, sem_last, sem_in, sem_out):

    def group_cols(g):
      return pl.ds(pl.multiple_of(g * GW, GW), GW)

    def head_cols(g, h):
      return pl.ds(pl.multiple_of((g + G * h) * DH, DH), DH)

    def slot(br, t):
      return t if br == 0 else NA + t


    def x_copy(br):
      return pltpu.make_async_copy((xa_h, xb_h)[br], x_buf.at[br], sem_x.at[br])

    def wq_copies(g, br):
      if br == 0:
        return [pltpu.make_async_copy(
            wqa_h.at[:, group_cols(g)], wq_buf.at[0, :, group_cols(g)], sem_k.at[0])]
      return [pltpu.make_async_copy(
          wqb_h.at[:, head_cols(g, h)], wq_buf.at[1, :, head_cols(g, h)], sem_k.at[NA])
              for h in range(REP)]

    def wo_copy(g, br):
      if br == 0:
        return pltpu.make_async_copy(
            woa_h.at[group_cols(g), :], woa_buf.at[group_cols(g), :], sem_v.at[0])
      return pltpu.make_async_copy(wob_h.at[:, g], wob_buf.at[:, g], sem_v.at[NA])

    def cache_copy(src, dst, sem, g, br, t, block, blocks, row, rows):
      j = slot(br, t)
      return pltpu.make_async_copy(
          src.at[pl.ds(t * P + block, blocks), g, pl.ds(row, rows)],
          dst.at[j, pl.ds(block, blocks), pl.ds(row, rows)], sem.at[j])

    def k_copies(g, br, t):
      return [cache_copy((ka_h, kb_h)[br], k_buf, sem_k, g, br, t, 0, P, s * SL, SL)
              for s in range(NSL)]

    def v_copies(g, br, t):
      copy = functools.partial(cache_copy, (va_h, vb_h)[br], v_buf, sem_v, g, br, t)
      kept = SK - STAGED[br]
      copies = []
      for row in range(0, SK - SL, SL):
        if row + SL <= kept:
          copies.append(copy(0, P, row, SL))
        else:
          if row < kept:
            copies.append(copy(P - 1, 1, row, kept - row))
          copies.append(copy(0, P - 1, row, SL))
      return copies

    def v_last_copy(g, br, t):
      return cache_copy((va_h, vb_h)[br], v_buf, sem_last, g, br, t, 0, P - 1, SK - SL, SL)

    def stage_in(g, br, t):
      n = g * NJ + slot(br, t)
      r = STAGED[br]
      return pltpu.make_async_copy(
          (va_h, vb_h)[br].at[t * P + P - 1, g, pl.ds(SK - r, r)],
          sbuf.at[n % (2 * DEPTH), pl.ds(0, r)], sem_in.at[n % DEPTH])

    def stage_out(g, br, t):
      j = slot(br, t)
      n = g * NJ + j
      r = STAGED[br]
      return pltpu.make_async_copy(
          sbuf.at[n % (2 * DEPTH), pl.ds(0, r)],
          v_buf.at[j, P - 1, pl.ds(SK - r, r)], sem_out.at[n % DEPTH])


    def on_first(t, fn):
      if isinstance(t, int):
        if t == 0:
          fn()
      else:
        pl.when(t == 0)(fn)

    def start_k(g, br, t):
      on_first(t, lambda: _start_all(wq_copies(g, br)))
      _start_all(k_copies(g, br, t))

    def start_v(g, br, t):
      on_first(t, lambda: wo_copy(g, br).start())
      _start_all(v_copies(g, br, t))

    def start_v_last(g, br, t):
      v_last_copy(g, br, t).start()

    def start_stage(g, br, t):
      stage_in(g, br, t).start()

    def forward_stage(g, br, t):
      stage_in(g, br, t).wait()
      stage_out(g, br, t).start()

    def later(g, br, t, d, fn):
      if br == 0:
        j = t + d
        if j < NA:
          fn(g, 0, j)
        else:
          fn(g, 1, j - NA)
        return
      pl.when(t + d < NB)(lambda: fn(g, 1, t + d))

      @pl.when(g + 1 < G)
      def _():
        for a in range(min(NA, d)):
          pl.when(t + d == NB + a)(functools.partial(fn, g + 1, 0, a))
        if d > NA:
          pl.when(t + d >= NJ)(lambda: fn(g + 1, 1, t + d - NJ))

    def wait_k(g, br, t):
      on_first(t, lambda: _wait_all(wq_copies(g, br)))
      _wait_all(k_copies(g, br, t))
      later(g, br, t, AHEAD, start_k)

    def wait_v(g, br, t):
      on_first(t, lambda: wo_copy(g, br).wait())
      _wait_all(v_copies(g, br, t))
      if br == 1:
        pl.when(jnp.logical_and(g == G - 1, t == NB - 1))(lambda: out_copy(False).start())
      later(g, br, t, AHEAD, start_v)
      stage_out(g, br, t).wait()
      later(g, br, t, DEPTH, forward_stage)
      later(g, br, t, 2 * DEPTH, start_stage)
      v_last_copy(g, br, t).wait()
      later(g, br, t, AHEAD, start_v_last)


    def q_proj(br, g, rows):
      if br == 0:
        w = wq_buf[0, :, group_cols(g)]
      else:
        w = jnp.concatenate([wq_buf[1, :, head_cols(g, h)] for h in range(REP)], axis=1)
      q = jnp.dot(x_buf[br, rows, :], w, preferred_element_type=jnp.float32)
      return (q * QSCALE).astype(jnp.bfloat16)

    def o_proj(br, g, rows, o):
      if br == 0:
        w = woa_buf[group_cols(g), :]
      else:
        w = jnp.concatenate([wob_buf[h, g] for h in range(REP)], axis=0)
      r = acc[br, rows, :] + jnp.dot(o, w, preferred_element_type=jnp.float32)
      acc[br, rows, :] = r
      obuf[rows, br * D:(br + 1) * D] = r.astype(jnp.bfloat16)

    def a_compute(g, t, c, carry):
      n = A_BATCH * SQ
      rows = pl.ds(pl.multiple_of(t * P * SQ + c * n, n), n)
      q = q_proj(0, g, rows)
      ps = []
      for i in range(A_BATCH):
        qi = jnp.concatenate(
            [q[i * SQ:(i + 1) * SQ, h * DH:(h + 1) * DH] for h in range(REP)], axis=0)
        ps.append(_softmax(_qk(qi, k_buf[t, c * A_BATCH + i])))
      outs = []
      for i in range(A_BATCH):
        o = _pv(*ps[i], v_buf[t, c * A_BATCH + i])
        outs.append(jnp.concatenate([o[h * SQ:(h + 1) * SQ] for h in range(REP)], axis=1))
      o_proj(0, g, rows, jnp.concatenate(outs, axis=0))
      return carry

    def b_step(g, t, carry):
      j = NA + t
      n = B_BATCH * SQ
      rows = pl.ds(pl.multiple_of(t * n, n), n)
      wait_k(g, 1, t)
      q = q_proj(1, g, rows)
      ps = [_softmax(_qk(q[i * SQ:(i + 1) * SQ, h * DH:(h + 1) * DH], k_buf[j, i * REP + h]))
            for i in range(B_BATCH) for h in range(REP)]
      wait_v(g, 1, t)
      outs = [jnp.concatenate(
          [_pv(*ps[i * REP + h], v_buf[j, i * REP + h]) for h in range(REP)], axis=1)
              for i in range(B_BATCH)]
      o_proj(1, g, rows, jnp.concatenate(outs, axis=0))
      return carry

    def group(g, carry):
      for t in range(NA):
        wait_k(g, 0, t)
        wait_v(g, 0, t)
        lax.fori_loop(0, P // A_BATCH, functools.partial(a_compute, g, t), 0)
      pl.when(g == 0)(lambda: x_copy(1).wait())
      lax.fori_loop(0, NB, functools.partial(b_step, g), 0)
      return carry

    first = [(0, 0, j) if j < NA else (0, 1, j - NA) for j in range(NJ)]
    for j in range(DEPTH):
      start_stage(*first[j])
    x_copy(0).start()
    for j in range(AHEAD):
      start_k(*first[j])
      start_v(*first[j])
      start_v_last(*first[j])
    x_copy(1).start()
    acc[...] = jnp.zeros_like(acc)
    for j in range(DEPTH):
      forward_stage(*first[j])
      start_stage(*first[j + DEPTH])
    x_copy(0).wait()

    lax.fori_loop(0, G, group, 0)
    out_copy(True).start()

  dma = pltpu.SemaphoreType.DMA
  pl.run_scoped(body, dma((2,)), dma((NJ,)), dma((NJ,)), dma((NJ,)), dma((DEPTH,)),
                dma((DEPTH,)))
  out_copy(False).wait()
  out_copy(True).wait()


@jax.jit
def pallas_concat_heads__gqa_block_cached__mha_block_cached__near_ridge_kernel(
    A_x: jax.Array,
    A_k_cache: jax.Array,
    A_v_cache: jax.Array,
    A_wq: jax.Array,
    A_wo: jax.Array,
    B_x: jax.Array,
    B_k_cache: jax.Array,
    B_v_cache: jax.Array,
    B_wq: jax.Array,
    B_wo: jax.Array,
):
  hbm = pl.BlockSpec(memory_space=pltpu.HBM)
  out = pl.pallas_call(
      _kernel,
      out_shape=jax.ShapeDtypeStruct((M, 2 * D), jnp.bfloat16),
      in_specs=[hbm] * 10,
      out_specs=hbm,
      scratch_shapes=[
          pltpu.VMEM((2, M, D), jnp.bfloat16),
          pltpu.VMEM((2, D, HQ * DH), jnp.bfloat16),
          pltpu.VMEM((HQ * DH, D), jnp.bfloat16),
          pltpu.VMEM((REP, G, DH, D), jnp.bfloat16),
          pltpu.VMEM((NJ, P, SK, DH), jnp.bfloat16),
          pltpu.VMEM((NJ, P, SK, DH), jnp.bfloat16),
          pltpu.VMEM((2, M, D), jnp.float32),
          pltpu.VMEM((M, 2 * D), jnp.bfloat16),
          pltpu.SMEM((2 * DEPTH, max(STAGED), DH), jnp.bfloat16),
          pltpu.SemaphoreType.DMA(()),
      ],
      compiler_params=pltpu.CompilerParams(
          vmem_limit_bytes=100 * 1024 * 1024, disable_bounds_checks=True),
  )(A_x.reshape(M, D), A_k_cache, A_v_cache, A_wq, A_wo,
    B_x.reshape(M, D),
    B_k_cache.reshape(B * REP, G, SK, DH), B_v_cache.reshape(B * REP, G, SK, DH),
    B_wq, B_wo.reshape(REP, G, DH, D))
  return out.reshape(B, SQ, 2 * D)
```

```python
import functools

import numpy as np

import jax
import jax.numpy as jnp
from jax import lax
import jax.experimental.pallas as pl
import jax.experimental.pallas.tpu as pltpu

B, SQ, D = 16, 32, 512
HQ, HKV, SK, DH = 32, 8, 512, 128
REP = HQ // HKV
G = HKV
GW = REP * DH
M = B * SQ

P = 8
NA = B // P
NB = B * REP // P
NJ = NA + NB
A_BATCH = 4
B_BATCH = P // REP
NSL = 4
SL = SK // NSL
AHEAD = 3
STAGED = (288, 272)
DEPTH = 3

QSCALE = float(DH ** -0.5 * np.log2(np.e))


def _start_all(copies):
  for cp in copies:
    cp.start()


def _wait_all(copies):
  for cp in copies:
    cp.wait()


def _qk(q, k):
  return lax.dot_general(q, k, (((1,), (1,)), ((), ())),
                         preferred_element_type=jnp.float32)


def _softmax(s):
  p = jnp.exp2(s - jnp.max(s, axis=-1, keepdims=True))
  return p.astype(jnp.bfloat16), 1.0 / jnp.sum(p, axis=-1, keepdims=True)


def _pv(p, r, v):
  return (jnp.dot(p, v, preferred_element_type=jnp.float32) * r).astype(jnp.bfloat16)


def _kernel(xa_h, ka_h, va_h, wqa_h, woa_h, xb_h, kb_h, vb_h, wqb_h, wob_h,
            out_h,
            x_buf, wq_buf, woa_buf, wob_buf, k_buf, v_buf, acc, obuf, sbuf,
            sem_o):

  def out_copy(last):
    n = B_BATCH * SQ
    rows = pl.ds(M - n, n) if last else pl.ds(0, M - n)
    return pltpu.make_async_copy(obuf.at[rows], out_h.at[rows], sem_o)

  def body(sem_x, sem_k, sem_v, sem_last, sem_in, sem_out):

    def group_cols(g):
      return pl.ds(pl.multiple_of(g * GW, GW), GW)

    def head_cols(g, h):
      return pl.ds(pl.multiple_of((g + G * h) * DH, DH), DH)

    def slot(br, t):
      return t if br == 0 else NA + t


    def x_copy(br):
      return pltpu.make_async_copy((xa_h, xb_h)[br], x_buf.at[br], sem_x.at[br])

    def wq_copies(g, br):
      if br == 0:
        return [pltpu.make_async_copy(
            wqa_h.at[:, group_cols(g)], wq_buf.at[0, :, group_cols(g)], sem_k.at[0])]
      return [pltpu.make_async_copy(
          wqb_h.at[:, head_cols(g, h)], wq_buf.at[1, :, head_cols(g, h)], sem_k.at[NA])
              for h in range(REP)]

    def wo_copy(g, br):
      if br == 0:
        return pltpu.make_async_copy(
            woa_h.at[group_cols(g), :], woa_buf.at[group_cols(g), :], sem_v.at[0])
      return pltpu.make_async_copy(wob_h.at[:, g], wob_buf.at[:, g], sem_v.at[NA])

    def cache_copy(src, dst, sem, g, br, t, block, blocks, row, rows):
      j = slot(br, t)
      return pltpu.make_async_copy(
          src.at[pl.ds(t * P + block, blocks), g, pl.ds(row, rows)],
          dst.at[j, pl.ds(block, blocks), pl.ds(row, rows)], sem.at[j])

    def k_copies(g, br, t):
      return [cache_copy((ka_h, kb_h)[br], k_buf, sem_k, g, br, t, 0, P, s * SL, SL)
              for s in range(NSL)]

    def v_copies(g, br, t):
      copy = functools.partial(cache_copy, (va_h, vb_h)[br], v_buf, sem_v, g, br, t)
      kept = SK - STAGED[br]
      copies = []
      for row in range(0, SK - SL, SL):
        if row + SL <= kept:
          copies.append(copy(0, P, row, SL))
        else:
          if row < kept:
            copies.append(copy(P - 1, 1, row, kept - row))
          copies.append(copy(0, P - 1, row, SL))
      return copies

    def v_last_copy(g, br, t):
      return cache_copy((va_h, vb_h)[br], v_buf, sem_last, g, br, t, 0, P - 1, SK - SL, SL)

    def stage_in(g, br, t):
      n = g * NJ + slot(br, t)
      r = STAGED[br]
      return pltpu.make_async_copy(
          (va_h, vb_h)[br].at[t * P + P - 1, g, pl.ds(SK - r, r)],
          sbuf.at[n % (2 * DEPTH), pl.ds(0, r)], sem_in.at[n % DEPTH])

    def stage_out(g, br, t):
      j = slot(br, t)
      n = g * NJ + j
      r = STAGED[br]
      return pltpu.make_async_copy(
          sbuf.at[n % (2 * DEPTH), pl.ds(0, r)],
          v_buf.at[j, P - 1, pl.ds(SK - r, r)], sem_out.at[n % DEPTH])


    def on_first(t, fn):
      if isinstance(t, int):
        if t == 0:
          fn()
      else:
        pl.when(t == 0)(fn)

    def start_k(g, br, t):
      on_first(t, lambda: _start_all(wq_copies(g, br)))
      _start_all(k_copies(g, br, t))

    def start_v(g, br, t):
      on_first(t, lambda: wo_copy(g, br).start())
      _start_all(v_copies(g, br, t))

    def start_v_last(g, br, t):
      v_last_copy(g, br, t).start()

    def start_stage(g, br, t):
      stage_in(g, br, t).start()

    def forward_stage(g, br, t):
      stage_in(g, br, t).wait()
      stage_out(g, br, t).start()

    def later(g, br, t, d, fn):
      assert NA <= d <= NB
      if br == 0:
        fn(g, 1, t + d - NA)
        return
      j = t + d
      more = g + 1 < G
      wraps = j >= NJ
      pl.when(jnp.logical_or(j < NB, jnp.logical_and(wraps, more)))(
          lambda: fn(jnp.where(wraps, g + 1, g), 1, jnp.where(wraps, j - NJ, j)))
      pl.when(jnp.logical_and(jnp.logical_and(j >= NB, j < NJ), more))(
          lambda: fn(g + 1, 0, j - NB))

    def wait_k(g, br, t):
      on_first(t, lambda: _wait_all(wq_copies(g, br)))
      _wait_all(k_copies(g, br, t))
      later(g, br, t, AHEAD, start_k)

    def wait_v(g, br, t):
      on_first(t, lambda: wo_copy(g, br).wait())
      _wait_all(v_copies(g, br, t))
      if br == 1:
        pl.when(jnp.logical_and(g == G - 1, t == NB - 1))(lambda: out_copy(False).start())
      later(g, br, t, AHEAD, start_v)
      stage_out(g, br, t).wait()
      later(g, br, t, DEPTH, forward_stage)
      later(g, br, t, 2 * DEPTH, start_stage)
      v_last_copy(g, br, t).wait()
      later(g, br, t, AHEAD, start_v_last)


    def q_proj(br, g, rows):
      if br == 0:
        w = wq_buf[0, :, group_cols(g)]
      else:
        w = jnp.concatenate([wq_buf[1, :, head_cols(g, h)] for h in range(REP)], axis=1)
      q = jnp.dot(x_buf[br, rows, :], w, preferred_element_type=jnp.float32)
      return (q * QSCALE).astype(jnp.bfloat16)

    def o_proj(br, g, rows, o):
      if br == 0:
        w = woa_buf[group_cols(g), :]
      else:
        w = jnp.concatenate([wob_buf[h, g] for h in range(REP)], axis=0)
      r = acc[br, rows, :] + jnp.dot(o, w, preferred_element_type=jnp.float32)
      acc[br, rows, :] = r
      obuf[rows, br * D:(br + 1) * D] = r.astype(jnp.bfloat16)

    def a_compute(g, t, c, carry):
      n = A_BATCH * SQ
      rows = pl.ds(pl.multiple_of(t * P * SQ + c * n, n), n)
      q = q_proj(0, g, rows)
      ps = []
      for i in range(A_BATCH):
        qi = jnp.concatenate(
            [q[i * SQ:(i + 1) * SQ, h * DH:(h + 1) * DH] for h in range(REP)], axis=0)
        ps.append(_softmax(_qk(qi, k_buf[t, c * A_BATCH + i])))
      outs = []
      for i in range(A_BATCH):
        o = _pv(*ps[i], v_buf[t, c * A_BATCH + i])
        outs.append(jnp.concatenate([o[h * SQ:(h + 1) * SQ] for h in range(REP)], axis=1))
      o_proj(0, g, rows, jnp.concatenate(outs, axis=0))
      return carry

    def b_step(g, t, carry):
      j = NA + t
      n = B_BATCH * SQ
      rows = pl.ds(pl.multiple_of(t * n, n), n)
      wait_k(g, 1, t)
      q = q_proj(1, g, rows)
      ps = [_softmax(_qk(q[i * SQ:(i + 1) * SQ, h * DH:(h + 1) * DH], k_buf[j, i * REP + h]))
            for i in range(B_BATCH) for h in range(REP)]
      wait_v(g, 1, t)
      outs = [jnp.concatenate(
          [_pv(*ps[i * REP + h], v_buf[j, i * REP + h]) for h in range(REP)], axis=1)
              for i in range(B_BATCH)]
      o_proj(1, g, rows, jnp.concatenate(outs, axis=0))
      return carry

    def a_step(g, t, carry):
      wait_k(g, 0, t)
      wait_v(g, 0, t)
      lax.fori_loop(0, P // A_BATCH, functools.partial(a_compute, g, t), 0)
      return carry

    def group(g, carry):
      lax.fori_loop(0, NA, functools.partial(a_step, g), 0)
      pl.when(g == 0)(lambda: x_copy(1).wait())
      lax.fori_loop(0, NB, functools.partial(b_step, g), 0)
      return carry

    first = [(0, 0, j) if j < NA else (0, 1, j - NA) for j in range(NJ)]
    for j in range(DEPTH):
      start_stage(*first[j])
    x_copy(0).start()
    for j in range(AHEAD):
      start_k(*first[j])
      start_v(*first[j])
      start_v_last(*first[j])
    x_copy(1).start()
    acc[...] = jnp.zeros_like(acc)
    for j in range(DEPTH):
      forward_stage(*first[j])
      start_stage(*first[j + DEPTH])
    x_copy(0).wait()

    lax.fori_loop(0, G, group, 0)
    out_copy(True).start()

  dma = pltpu.SemaphoreType.DMA
  pl.run_scoped(body, dma((2,)), dma((NJ,)), dma((NJ,)), dma((NJ,)), dma((DEPTH,)),
                dma((DEPTH,)))
  out_copy(False).wait()
  out_copy(True).wait()


@jax.jit
def pallas_concat_heads__gqa_block_cached__mha_block_cached__near_ridge_kernel(
    A_x: jax.Array,
    A_k_cache: jax.Array,
    A_v_cache: jax.Array,
    A_wq: jax.Array,
    A_wo: jax.Array,
    B_x: jax.Array,
    B_k_cache: jax.Array,
    B_v_cache: jax.Array,
    B_wq: jax.Array,
    B_wo: jax.Array,
):
  hbm = pl.BlockSpec(memory_space=pltpu.HBM)
  out = pl.pallas_call(
      _kernel,
      out_shape=jax.ShapeDtypeStruct((M, 2 * D), jnp.bfloat16),
      in_specs=[hbm] * 10,
      out_specs=hbm,
      scratch_shapes=[
          pltpu.VMEM((2, M, D), jnp.bfloat16),
          pltpu.VMEM((2, D, HQ * DH), jnp.bfloat16),
          pltpu.VMEM((HQ * DH, D), jnp.bfloat16),
          pltpu.VMEM((REP, G, DH, D), jnp.bfloat16),
          pltpu.VMEM((NJ, P, SK, DH), jnp.bfloat16),
          pltpu.VMEM((NJ, P, SK, DH), jnp.bfloat16),
          pltpu.VMEM((2, M, D), jnp.float32),
          pltpu.VMEM((M, 2 * D), jnp.bfloat16),
          pltpu.SMEM((2 * DEPTH, max(STAGED), DH), jnp.bfloat16),
          pltpu.SemaphoreType.DMA(()),
      ],
      compiler_params=pltpu.CompilerParams(
          vmem_limit_bytes=100 * 1024 * 1024, disable_bounds_checks=True),
  )(A_x.reshape(M, D), A_k_cache, A_v_cache, A_wq, A_wo,
    B_x.reshape(M, D),
    B_k_cache.reshape(B * REP, G, SK, DH), B_v_cache.reshape(B * REP, G, SK, DH),
    B_wq, B_wo.reshape(REP, G, DH, D))
  return out.reshape(B, SQ, 2 * D)
```
